```python
import os as _os
_os.environ.setdefault("JAX_PLATFORMS", "cpu")
import jax
import jax.numpy as jnp

def _softmax(x, axis=-1):
    return jax.nn.softmax(x, axis=axis)
def _gelu(x):
    return jax.nn.gelu(x, approximate=True)
def _silu(x):
    return jax.nn.silu(x)
def _sigmoid(x):
    return jax.nn.sigmoid(x)
def _layernorm(x, axis=-1, eps=1e-5):
    m = jnp.mean(x, axis=axis, keepdims=True)
    v = jnp.var(x, axis=axis, keepdims=True)
    return (x - m) / jnp.sqrt(v + eps)
def _scatter_add(tgt, idx, src, axis=0):
    return tgt.at[idx].add(src)
def _segment_sum(src, seg, n):
    return jax.ops.segment_sum(src, seg, n)
class _Rng:
    def __init__(self, key):
        self._k = key
    def _next(self):
        self._k, sub = jax.random.split(self._k)
        return sub
    def normal(self, shape):
        return jax.random.normal(self._next(), shape, dtype=jnp.bfloat16)
    def randint(self, lo, hi, shape):
        return jax.random.randint(self._next(), shape, lo, hi, dtype=jnp.int32)
    def uniform(self, shape, lo=0.0, hi=1.0):
        return jax.random.uniform(self._next(), shape, jnp.bfloat16, lo, hi)
    def permutation(self, n):
        return jax.random.permutation(self._next(), n)


kernel_name = 'concat_heads__sliding_local_dilated__compressed_kv_cla__prompt'

def setup_inputs():
    _rng = _Rng(jax.random.key(int.from_bytes(__import__("os").urandom(4), "little")))
    _w = (lambda a: (lambda t: t.astype(jnp.bfloat16) if jnp.issubdtype(t.dtype, jnp.floating) else t)(jnp.asarray(a)))
    def _A_setup():
        B, S, D = 1, 2048, 640
        return {
            "x": _w((lambda *s: _rng.normal(s) * 0.2)(B, S, D)),
            "wqkv": _w((lambda *s: _rng.normal(s) * 0.2)(D, 3 * D)),
            "wo": _w((lambda *s: _rng.normal(s) * 0.05)(D, D)),
        }
    _A_in = _A_setup()

    def _B_setup():
        B, H, Sq, Sk, D, M = 1, 32, 2048, 2048, 128, 640
        Dc = 4 * D
        return {
            "x": _w((lambda *s: _rng.normal(s) * 0.8)(B, Sq, M)),
            "c_kv": _w((lambda *s: _rng.normal(s) * 0.8)(B, Sk, Dc)),
            "w_q": _w((lambda *s: _rng.normal(s) * 1.6)(M, H, D) * (M ** -0.5)),
            "w_uk": _w((lambda *s: _rng.normal(s) * 1.6)(Dc, H, D) * (Dc ** -0.5)),
            "w_uv": _w((lambda *s: _rng.normal(s) * 0.8)(Dc, H, D) * (Dc ** -0.5)),
            "w_o": _w((lambda *s: _rng.normal(s) * 0.8)(H, D, M) * ((H * D) ** -0.5)),
        }
    _B_in = _B_setup()

    return {
        "A_x": _A_in["x"],
        "A_wqkv": _A_in["wqkv"],
        "A_wo": _A_in["wo"],
        "B_x": _B_in["x"],
        "B_c_kv": _B_in["c_kv"],
        "B_w_q": _B_in["w_q"],
        "B_w_uk": _B_in["w_uk"],
        "B_w_uv": _B_in["w_uv"],
        "B_w_o": _B_in["w_o"],
    }

def reference(A_x, A_wqkv, A_wo, B_x, B_c_kv, B_w_q, B_w_uk, B_w_uv, B_w_o):
    def _A_ref(x, wqkv, wo):
        B, S, D = x.shape
        H = 32; Dh = D // H
        W, dil = 8, 2
        qkv = (lambda x, *d: x.transpose(*d))((x @ wqkv).reshape(B, S, 3, H, Dh), 2, 0, 3, 1, 4)
        q, k, v = qkv[0], qkv[1], qkv[2]
        scale = Dh ** -0.5
        pos = jnp.arange(S)
        off = jnp.arange(W) * dil
        idx = pos[:, None] - off[None, :]
        mask = idx >= 0
        idx_c = jnp.where(mask, idx, 0).reshape(-1)
        kg = k[:, :, idx_c, :].reshape(B, H, S, W, Dh)
        vg = v[:, :, idx_c, :].reshape(B, H, S, W, Dh)
        logits = jnp.einsum("bhsd,bhswd->bhsw", q, kg) * scale
        logits = jnp.where(mask[None, None, :, :], logits, -1e9)
        attn = _softmax(logits, axis=-1)
        o = jnp.einsum("bhsw,bhswd->bhsd", attn, vg)
        return (lambda x, *d: x.transpose(*d))(o, 0, 2, 1, 3).reshape(B, S, D) @ wo

    def _B_ref(x, c_kv, w_q, w_uk, w_uv, w_o):
        B, Sq, M = x.shape[0], x.shape[1], x.shape[2]
        Sk = c_kv.shape[1]
        H, D = w_q.shape[1], w_q.shape[2]
        q = jnp.einsum("bqm,mhd->bhqd", x, w_q)
        k = jnp.einsum("bkc,chd->bhkd", c_kv, w_uk)
        v = jnp.einsum("bkc,chd->bhkd", c_kv, w_uv)
        scores = jnp.einsum("bhqd,bhkd->bhqk", q, k) * (D ** -0.5)
        off = Sk - Sq
        qi = jnp.arange(Sq)[:, None]
        kj = jnp.arange(Sk)[None, :]
        cmask = kj <= (qi + off)
        scores = jnp.where(cmask[None, None], scores, -1e9)
        p = _softmax(scores, axis=-1)
        ctx = jnp.einsum("bhqk,bhkd->bhqd", p, v)
        return jnp.einsum("bhqd,hdm->bqm", ctx, w_o)

    a = _A_ref(A_x, A_wqkv, A_wo)
    b = _B_ref(B_x, B_c_kv, B_w_q, B_w_uk, B_w_uv, B_w_o)
    return jnp.concatenate([a, b], axis=-1)
```

```python
import math

import jax
import jax.numpy as jnp
from jax import lax
import jax.experimental.pallas as pl
import jax.experimental.pallas.tpu as pltpu

bf16, f32, u32 = jnp.bfloat16, jnp.float32, jnp.uint32
NT = (((1,), (1,)), ((), ()))
NEG = -1e30
LOG2E = math.log2(math.e)

S = 2048
DM = 640
NL = DM // 128
HA, DH, WIN, DIL = 32, 20, 8, 2
PAD = 16
TA = 512
NA = S // TA
NA1 = 2
H, D, C = 32, 128, 512
G = 8
NG = H // G
T = 128
ASCALE = DH ** -0.5 * LOG2E
QSCALE = D ** -0.5 * LOG2E

DEFAULT = dict(
    TQ=256,
    TP=512,
    RB=32,
    hps=2,
    RCA=16,
    asb='64-64-64-64-64-64-64-64',
    oc='0-256-384-512',
    aorder=('K0,Q0,V0,K1,Q1,V1,K2,Q2,V2,K3,Q3,V3,K4,K5,Q4,V4,O0,Q5,V5,O1,Q6,K6,V6,O2,Q7,V7,K7,O3,O4,O5,O7,O6'),
    order=('Y:K1a,Q3a,K0a,K2a,K3a,Q1a,QK7a,Q2a,QK6a,V0a,V1a,QK5a,V3a,Q0a,V2a,QK4a,PV7a,PV6a,OP7a,QK3a,PV5a,'
           'OP6a,K0b,QK2a,PV4a,OP5a,QK1a,PV3a,QK0a,OP4a,K1b,PV2a,OP2a,OP3a,PV0a,K2b,Q1b,Q3b,K3b,QK7b,Q0b,'
           'OP0a,PV1a,Q2b,QK6b,V1b,V0b,V2b,OP1a,QK5b,V3b,PV7b,QK4b,PV6b,QK0b,OP7b,PV5b,QK3b,OP6b,QK2b,PV4b,'
           'OP5b,QK1b,PV3b,OP4b,OP3b,PV2b,PV1b,PV0b,OP1b,OP2b,OP0b'),
)


def _pk(x):
    return pltpu.bitcast(x, u32)


def _up(x):
    return pltpu.bitcast(x, bf16)


def b_order(name, hps):
    o = []
    toks = name[2:].split(',')
    if name[0] == 'X':
        toks = [t + 'abcdefgh'[hi] for hi in range(hps) for t in toks]
    for tok in toks:
        hi = 'abcdefgh'.index(tok[-1])
        tok = tok[:-1]
        kind = tok.rstrip('0123456789')
        o.append((kind, int(tok[len(kind):]), hi))
    return o


def make_kernel(cfg):
    cfg = {**DEFAULT, **cfg}
    TQ, TP, RB = cfg['TQ'], cfg['TP'], cfg['RB']
    cfg['ocuts'] = [int(v) for v in cfg['oc'].split('-')]
    RCA = cfg['RCA']
    hps = cfg['hps']
    NB = H // hps
    NSTEPS = NA + NB

    def _kernel(xa_hbm, wqkv_hbm, woa_hbm, xb_hbm, c_hbm, wq_hbm, wk_hbm, wv_hbm, wob_hbm,
                out_hbm,
                xa_v, wqkv_v, woa_v, wt_f, wo_f, wt_p, wo_p, qa_s, ka_s, va_s, oa_s, outa_v,
                xb_v, c_v, wq_v, wk_v, wv_v, wob_v, wqT, wkT, wvT, acc_ref, q_ss, k_ss, v_ss, p_ss,
                xb32, c32, wo_hs, outb_v,
                sem):
        step = pl.program_id(0)
        is_a = jnp.logical_or(step < NA1, step >= NA1 + NB)
        ablk = jnp.clip(jnp.where(step < NA1, step, step - NB), 0, NA - 1)
        h0 = jnp.clip(step - NA1, 0, NB - 1) * hps

        def cp_xa(i):
            return pltpu.make_async_copy(xa_hbm.at[0, pl.ds(i * TA, TA), :], xa_v.at[i], sem.at[i])

        def cp_wqkv(j):
            return pltpu.make_async_copy(wqkv_hbm.at[pl.ds(j * 128, 128), :], wqkv_v.at[j], sem.at[31 + j])

        def cp_woa():
            return pltpu.make_async_copy(woa_hbm, woa_v, sem.at[7])

        def cp_xb():
            return pltpu.make_async_copy(xb_hbm.at[0], xb_v, sem.at[8])

        def cp_c():
            return pltpu.make_async_copy(c_hbm.at[0], c_v, sem.at[9])

        def cp_group(g):
            return [
                pltpu.make_async_copy(wk_hbm.at[:, pl.ds(g * G, G), :], wk_v.at[g], sem.at[14 + g]),
                pltpu.make_async_copy(wq_hbm.at[:, pl.ds(g * G, G), :], wq_v.at[g], sem.at[10 + g]),
                pltpu.make_async_copy(wv_hbm.at[:, pl.ds(g * G, G), :], wv_v.at[g], sem.at[18 + g]),
            ]

        def cp_wob(g):
            return pltpu.make_async_copy(wob_hbm.at[pl.ds(g * G, G)], wob_v.at[pl.ds(g * G, G)], sem.at[22 + g])

        ocuts = cfg['ocuts']
        last = step == NSTEPS - 1

        def cp_outa(i):
            start = i * TA if isinstance(i, int) else pl.multiple_of(i * TA, TA)
            return pltpu.make_async_copy(outa_v.at[i], out_hbm.at[0, pl.ds(start, TA), pl.ds(0, DM)],
                                         sem.at[26 + i])

        def cp_outa_last(part):
            lo, hi = ocuts[part], ocuts[part + 1]
            return pltpu.make_async_copy(outa_v.at[NA - 1, pl.ds(lo, hi - lo), :],
                                         out_hbm.at[0, pl.ds((NA - 1) * TA + lo, hi - lo), pl.ds(0, DM)],
                                         sem.at[36 + part])

        def cp_outb():
            return pltpu.make_async_copy(outb_v, out_hbm.at[0, :, pl.ds(DM, DM)], sem.at[30])

        wsets = {'K': (wk_v, wkT, C), 'Q': (wq_v, wqT, DM), 'V': (wv_v, wvT, C)}

        def relayout_unit(kind, g, g8, r0, half_r0):
            src, dst, _ = wsets[kind]
            dst[pl.ds(g8, G), pl.ds(half_r0, 8), :] = _pk(jnp.swapaxes(src[g, pl.ds(r0, 16), :, :], 0, 1))

        def prologue0():
            for j in range(NL):
                cp_wqkv(j).start()
            cp_woa().start()
            cp_xa(0).start()
            cp_xa(1).start()
            for cp in cp_group(0):
                cp.start()
            cp_c().start()
            cp_xb().start()
            cp_wob(0).start()
            for cp in cp_group(1):
                cp.start()
            ka_s[:, TA:TA + PAD, :] = jnp.zeros((NL, PAD, 128), f32)
            va_s[:, TA:TA + PAD, :] = jnp.zeros((NL, PAD, 128), f32)
            acc_ref[...] = jnp.zeros_like(acc_ref)
            for mt in range(NL):
                cp_wqkv(mt).wait()
                for lt in range(3 * NL):
                    blk = wqkv_v[mt, :, lt * 128:(lt + 1) * 128]
                    wt_f[mt % 2, lt * 128:(lt + 1) * 128, :] = blk.T.astype(f32)
                for j in range(3):
                    for d in range(DH):
                        val = wt_f[mt % 2, pl.ds(j * DM + d, HA, stride=DH), :].astype(bf16)
                        wt_p[(j * DM + d * HA) // 2:(j * DM + (d + 1) * HA) // 2, mt * 128:(mt + 1) * 128] = _pk(val)
            cp_woa().wait()
            for mt in range(NL):
                wo_f[mt] = woa_v[:, mt * 128:(mt + 1) * 128].astype(f32)
            for d in range(DH):
                for mt in range(NL):
                    val = wo_f[mt, pl.ds(d, HA, stride=DH), :].astype(bf16)
                    wo_p[d * HA // 2:(d + 1) * HA // 2, mt * 128:(mt + 1) * 128] = _pk(val)
            cp_xa(0).wait()

        def a_events():
            pl.when(step == 0)(prologue0)

            @pl.when(step == 1)
            def _():
                cp_xa(1).wait()

            @pl.when(step == NA1 + NB)
            def _():
                outb_v[...] = acc_ref[...].astype(bf16)
                cp_outb().start()
                for i in range(NA1, NA):
                    cp_xa(i).wait()

        def a_post():
            @pl.when(jnp.logical_not(last))
            def _():
                cp_outa(ablk).start()

            @pl.when(last)
            def _():
                cp_outa_last(len(ocuts) - 2).start()
                cp_outb().wait()
                for i in range(NA - 1):
                    cp_outa(i).wait()
                for part in range(len(ocuts) - 1):
                    cp_outa_last(part).wait()

        def b_events():
            @pl.when(h0 % G == 0)
            def _():
                for g in range(NG):
                    @pl.when(h0 == g * G)
                    def _(g=g):
                        if g == 0:
                            for cp in cp_group(0):
                                cp.wait()
                            cp_c().wait()
                            cp_xb().wait()
                            units = [(kind, r0) for kind in 'KQV' for r0 in range(0, wsets[kind][2], 16)]
                            per = -(-S // len(units) // 16) * 16
                            r = 0
                            for kind, r0 in units:
                                relayout_unit(kind, 0, 0, r0, r0 // 2)
                                if r < S:
                                    e = min(S, r + per)
                                    xb32[r // 2:e // 2, :] = _pk(xb_v[r:e, :])
                                    c32[r // 2:e // 2, :] = _pk(c_v[r:e, :])
                                    r = e
                        cp_wob(g).wait()
                        if g + 1 < NG:
                            for cp in cp_group(g + 1):
                                cp.wait()
                            cp_wob(g + 1).start()
                        if g + 2 < NG:
                            for cp in cp_group(g + 2):
                                cp.start()
                        if g == NG - 1:
                            for i in range(NA1, NA):
                                cp_xa(i).start()

        @pl.when(is_a)
        def _():
            a_events()
            cuts = [0]
            for v in cfg['asb'].split('-'):
                cuts.append(cuts[-1] + int(v))
            assert cuts[-1] == TA
            ka_s[:, 0:PAD, :] = ka_s[:, TA:TA + PAD, :]
            va_s[:, 0:PAD, :] = va_s[:, TA:TA + PAD, :]
            xcache = {}
            aparts = {'K': (1, ka_s, PAD), 'Q': (0, qa_s, 0), 'V': (2, va_s, PAD)}

            def proj(kind, b):
                lo, hi = cuts[b], cuts[b + 1]
                part, dst, off = aparts[kind]
                if b not in xcache:
                    xcache[b] = xa_v[ablk, lo:hi, :]
                x = xcache[b]
                w = _up(wt_p[part * DM // 2:(part + 1) * DM // 2, :])
                y = lax.dot_general(x, w, NT, preferred_element_type=f32)
                if part == 0:
                    y = y * ASCALE
                for j in range(NL):
                    dst[j, off + lo:off + hi, :] = y[:, j * 128:(j + 1) * 128]

            def attn(b):
                for r0 in range(cuts[b], cuts[b + 1], RCA):
                    q = [qa_s[j, r0:r0 + RCA, :] for j in range(NL)]
                    lg = []
                    for w in range(WIN):
                        st = PAD + r0 - DIL * w
                        a = None
                        for j in range(NL):
                            pr = q[j] * ka_s[j, st:st + RCA, :]
                            a = pr if a is None else a + pr
                        a = a + pltpu.roll(a, 64, axis=1)
                        a = a + pltpu.roll(a, 32, axis=1)
                        if r0 < PAD and w > 0:
                            grow = ablk * TA + r0 + lax.broadcasted_iota(jnp.int32, (RCA, 128), 0)
                            a = jnp.where(grow >= DIL * w, a, NEG)
                        lg.append(a)
                    m = lg[0]
                    for w in range(1, WIN):
                        m = jnp.maximum(m, lg[w])
                    ps = [jnp.exp2(lg[w] - m) for w in range(WIN)]
                    l = ps[0]
                    for w in range(1, WIN):
                        l = l + ps[w]
                    inv = 1.0 / l
                    for j in range(NL):
                        a = None
                        for w in range(WIN):
                            st = PAD + r0 - DIL * w
                            pr = ps[w] * va_s[j, st:st + RCA, :]
                            a = pr if a is None else a + pr
                        oa_s[r0:r0 + RCA, j * 128:(j + 1) * 128] = (a * inv).astype(bf16)

            def op(b):
                r = slice(cuts[b], cuts[b + 1])
                outa_v[ablk, r, :] = jnp.dot(oa_s[r, :], _up(wo_p[...]), preferred_element_type=f32).astype(bf16)

            nsb = len(cuts) - 1
            done = set()
            att_done = 0
            ops_done = set()
            for tok in cfg['aorder'].split(','):
                kind, b = tok[0], int(tok[1:])
                if kind == 'O':
                    op(b)
                    ops_done.add(b)
                    for part in range(len(ocuts) - 2):
                        need = [bb for bb in range(nsb) if cuts[bb] < ocuts[part + 1] and cuts[bb + 1] > ocuts[part]]
                        if b in need and all(bb in ops_done for bb in need):
                            pl.when(last)(lambda part=part: cp_outa_last(part).start())
                else:
                    proj(kind, b)
                    done.add((kind, b))
                    while att_done < nsb and all((kk, bb) in done for kk in 'KV' for bb in range(max(att_done - 1, 0), att_done + 1)) \
                            and ('Q', att_done) in done:
                        attn(att_done)
                        att_done += 1
            a_post()

        @pl.when(jnp.logical_not(is_a))
        def _():
            b_events()
            nt = TQ // T
            npj = S // TP
            row = lax.broadcasted_iota(jnp.int32, (T, T), 0)
            col = lax.broadcasted_iota(jnp.int32, (T, T), 1)
            dmask = col <= row

            def head(hi):
                h = h0 + hi
                wo_h = wo_hs.at[hi]
                q_s, k_s, v_s, p_s = q_ss[hi], k_ss[hi], v_ss[hi], p_ss[hi]
                wo_h[...] = _pk(wob_v[h])
                gn = jnp.minimum(h // G + 1, NG - 1)
                rp = h % G
                cnt = {'K': 0, 'Q': 0, 'V': 0}

                def ld(ref, lo, hi):
                    return _up(ref[lo // 2:hi // 2, :])

                def proj(kind, j):
                    _, wT, rows = wsets[kind]
                    lo, hi = j * TP, (j + 1) * TP
                    w = _up(wT[h])
                    y = jnp.dot(ld(xb32 if kind == 'Q' else c32, lo, hi), w, preferred_element_type=f32)
                    if kind == 'Q':
                        y = y * QSCALE
                    dst = {'K': k_s, 'Q': q_s, 'V': v_s}[kind]
                    dst[lo // 2:hi // 2, :] = _pk(y.astype(bf16))
                    n = rows // G
                    units = n // 16
                    c = cnt[kind]
                    cnt[kind] += 1
                    for u in range((units * c) // npj, (units * (c + 1)) // npj):
                        relayout_unit(kind, gn, gn * G, pl.multiple_of(rp * n + u * 16, 16),
                                      pl.multiple_of(rp * (n // 2) + u * 8, 8))

                def qk_softmax(i):
                    base = i * TQ
                    q = ld(q_s, base, base + TQ)
                    n0 = base + T
                    s0 = lax.dot_general(q, ld(k_s, 0, n0), NT, preferred_element_type=f32)
                    extra = {}
                    for t in range(1, nt):
                        extra[t] = lax.dot_general(q[t * T:], ld(k_s, base + t * T, base + (t + 1) * T), NT,
                                                   preferred_element_type=f32)
                    ls = []
                    for t in range(nt):
                        for r0 in range(t * T, (t + 1) * T, RB):
                            rl = r0 - t * T
                            parts = []
                            dm = dmask[rl:rl + RB]
                            if t == 0:
                                if base > 0:
                                    parts.append(s0[r0:r0 + RB, 0:base])
                                parts.append(jnp.where(dm, s0[r0:r0 + RB, base:n0], NEG))
                            else:
                                parts.append(s0[r0:r0 + RB])
                                for u in range(1, t + 1):
                                    e = extra[u][r0 - u * T:r0 - u * T + RB]
                                    if u == t:
                                        e = jnp.where(dm, e, NEG)
                                    parts.append(e)
                            s = jnp.concatenate(parts, axis=1) if len(parts) > 1 else parts[0]
                            m = jnp.max(s, axis=1, keepdims=True)
                            p = jnp.exp2(s - m)
                            ls.append(jnp.sum(p, axis=1, keepdims=True))
                            p_s[i][r0:r0 + RB, 0:base + (t + 1) * T] = p.astype(bf16)
                    return jnp.concatenate(ls, axis=0)

                def pv(i, l):
                    base = i * TQ
                    n0 = base + T
                    acc = jnp.dot(p_s[i][:, 0:n0], ld(v_s, 0, n0), preferred_element_type=f32)
                    accs = [acc[t * T:(t + 1) * T] for t in range(nt)]
                    for u in range(1, nt):
                        e = jnp.dot(p_s[i][u * T:TQ, base + u * T:base + (u + 1) * T],
                                    ld(v_s, base + u * T, base + (u + 1) * T), preferred_element_type=f32)
                        for t in range(u, nt):
                            accs[t] = accs[t] + e[(t - u) * T:(t - u + 1) * T]
                    acc = jnp.concatenate(accs, axis=0) if nt > 1 else accs[0]
                    return (acc * (1.0 / l)).astype(bf16)

                def op(i, ctx):
                    r = slice(i * TQ, (i + 1) * TQ)
                    acc_ref[r, :] += jnp.dot(ctx, _up(wo_h[...]), preferred_element_type=f32)

                ls, ctxs = {}, {}

                def run(kind, j):
                    if kind in 'KQV':
                        proj(kind, j)
                    elif kind == 'QK':
                        ls[j] = qk_softmax(j)
                    elif kind == 'PV':
                        ctxs[j] = pv(j, ls[j])
                    else:
                        op(j, ctxs[j])
                return run

            runs = [head(hi) for hi in range(hps)]
            for kind, j, hi in b_order(cfg['order'], hps):
                runs[hi](kind, j)

    def fn(A_x, A_wqkv, A_wo, B_x, B_c_kv, B_w_q, B_w_uk, B_w_uv, B_w_o):
        any_spec = pl.BlockSpec(memory_space=pl.ANY)
        V = pltpu.VMEM
        scratch = [
            V((NA, TA, DM), bf16),
            V((NL, 128, 3 * DM), bf16),
            V((DM, DM), bf16),
            V((2, 3 * DM, 128), f32),
            V((NL, DM, 128), f32),
            V((3 * DM // 2, DM), u32),
            V((DM // 2, DM), u32),
            V((NL, TA, 128), f32),
            V((NL, TA + PAD, 128), f32),
            V((NL, TA + PAD, 128), f32),
            V((TA, DM), bf16),
            V((NA, TA, DM), bf16),
            V((S, DM), bf16),
            V((S, C), bf16),
            V((NG, DM, G, D), bf16),
            V((NG, C, G, D), bf16),
            V((NG, C, G, D), bf16),
            V((H, D, DM), bf16),
            V((H, DM // 2, D), u32),
            V((H, C // 2, D), u32),
            V((H, C // 2, D), u32),
            V((S, DM), f32),
            [V((S // 2, D), u32)] * hps,
            [V((S // 2, D), u32)] * hps,
            [V((S // 2, D), u32)] * hps,
            [[V((TQ, (i + 1) * TQ), bf16) for i in range(S // TQ)] for _ in range(hps)],
            V((S // 2, DM), u32),
            V((S // 2, C), u32),
            V((hps, D // 2, DM), u32),
            V((S, DM), bf16),
            pltpu.SemaphoreType.DMA((36 + len(cfg['ocuts']) - 1,)),
        ]
        return pl.pallas_call(
            _kernel,
            grid=(NSTEPS,),
            in_specs=[any_spec] * 9,
            out_specs=any_spec,
            out_shape=jax.ShapeDtypeStruct((1, S, 2 * DM), bf16),
            scratch_shapes=scratch,
            compiler_params=pltpu.CompilerParams(
                dimension_semantics=("arbitrary",),
                vmem_limit_bytes=110 * 1024 * 1024,
            ),
        )(A_x, A_wqkv, A_wo, B_x, B_c_kv, B_w_q, B_w_uk, B_w_uv, B_w_o)

    return fn


_FN = make_kernel({})


@jax.jit
def pallas_concat_heads__sliding_local_dilated__compressed_kv_cla__prompt_kernel(
    A_x: jax.Array,
    A_wqkv: jax.Array,
    A_wo: jax.Array,
    B_x: jax.Array,
    B_c_kv: jax.Array,
    B_w_q: jax.Array,
    B_w_uk: jax.Array,
    B_w_uv: jax.Array,
    B_w_o: jax.Array,
):
    return _FN(A_x, A_wqkv, A_wo, B_x, B_c_kv, B_w_q, B_w_uk, B_w_uv, B_w_o)
```
